```python
import os as _os
_os.environ.setdefault("JAX_PLATFORMS", "cpu")
import jax
import jax.numpy as jnp

def _softmax(x, axis=-1):
    return jax.nn.softmax(x, axis=axis)
def _gelu(x):
    return jax.nn.gelu(x, approximate=True)
def _silu(x):
    return jax.nn.silu(x)
def _sigmoid(x):
    return jax.nn.sigmoid(x)
def _layernorm(x, axis=-1, eps=1e-5):
    m = jnp.mean(x, axis=axis, keepdims=True)
    v = jnp.var(x, axis=axis, keepdims=True)
    return (x - m) / jnp.sqrt(v + eps)
def _scatter_add(tgt, idx, src, axis=0):
    return tgt.at[idx].add(src)
def _segment_sum(src, seg, n):
    return jax.ops.segment_sum(src, seg, n)
class _Rng:
    def __init__(self, key):
        self._k = key
    def _next(self):
        self._k, sub = jax.random.split(self._k)
        return sub
    def normal(self, shape):
        return jax.random.normal(self._next(), shape, dtype=jnp.bfloat16)
    def randint(self, lo, hi, shape):
        return jax.random.randint(self._next(), shape, lo, hi, dtype=jnp.int32)
    def uniform(self, shape, lo=0.0, hi=1.0):
        return jax.random.uniform(self._next(), shape, jnp.bfloat16, lo, hi)
    def permutation(self, n):
        return jax.random.permutation(self._next(), n)


kernel_name = 'concat_heads__gqa_block_cached__sliding_block_cached__decode'

def setup_inputs():
    _rng = _Rng(jax.random.key(int.from_bytes(__import__("os").urandom(4), "little")))
    _w = (lambda a: (lambda t: t.astype(jnp.bfloat16) if jnp.issubdtype(t.dtype, jnp.floating) else t)(jnp.asarray(a)))
    def _A_setup():
        B, Sq, D = 1, 1, 576
        Hq, Hkv, Sk, Dh = 32, 16, 8192, 128
        assert Hq % Hkv == 0, (Hq, Hkv)
        return {
            "x": _w((lambda *s: _rng.normal(s) * 0.8)(B, Sq, D)),
            "k_cache": _w((lambda *s: _rng.normal(s) * 0.8)(B, Hkv, Sk, Dh)),
            "v_cache": _w((lambda *s: _rng.normal(s) * 0.05)(B, Hkv, Sk, Dh)),
            "wq": _w((lambda *s: _rng.normal(s) * 0.8)(D, Hq * Dh) * (D ** -0.5)),
            "wo": _w((lambda *s: _rng.normal(s) * 0.05)(Hq * Dh, D) * ((Hq * Dh) ** -0.5)),
        }
    _A_in = _A_setup()

    def _B_setup():
        B, Sq, D = 1, 1, 576
        Hq, Hkv, Sk, Dh = 32, 16, 8192, 128
        assert Hq % Hkv == 0, (Hq, Hkv)
        return {
            "x": _w((lambda *s: _rng.normal(s) * 0.8)(B, Sq, D)),
            "k_cache": _w((lambda *s: _rng.normal(s) * 0.8)(B, Hkv, Sk, Dh)),
            "v_cache": _w((lambda *s: _rng.normal(s) * 0.05)(B, Hkv, Sk, Dh)),
            "wq": _w((lambda *s: _rng.normal(s) * 0.8)(D, Hq * Dh) * (D ** -0.5)),
            "wo": _w((lambda *s: _rng.normal(s) * 0.05)(Hq * Dh, D) * ((Hq * Dh) ** -0.5)),
        }
    _B_in = _B_setup()

    return {
        "A_x": _A_in["x"],
        "A_k_cache": _A_in["k_cache"],
        "A_v_cache": _A_in["v_cache"],
        "A_wq": _A_in["wq"],
        "A_wo": _A_in["wo"],
        "B_x": _B_in["x"],
        "B_k_cache": _B_in["k_cache"],
        "B_v_cache": _B_in["v_cache"],
        "B_wq": _B_in["wq"],
        "B_wo": _B_in["wo"],
    }

def reference(A_x, A_k_cache, A_v_cache, A_wq, A_wo, B_x, B_k_cache, B_v_cache, B_wq, B_wo):
    def _A_ref(x, k_cache, v_cache, wq, wo):
        B, Sq, D = x.shape
        Hq, Dh = 32, 128
        Hkv = k_cache.shape[1]
        rep = Hq // Hkv
        q = (lambda x, *d: x.transpose(*d))((x @ wq).reshape(B, Sq, Hq, Dh), 0, 2, 1, 3)
        k = jnp.repeat(k_cache, rep, axis=1)
        v = jnp.repeat(v_cache, rep, axis=1)
        scores = jnp.einsum("bhqd,bhkd->bhqk", q, k) * (Dh ** -0.5)
        p = _softmax(scores, axis=-1)
        o = jnp.einsum("bhqk,bhkd->bhqd", p, v)
        return (lambda x, *d: x.transpose(*d))(o, 0, 2, 1, 3).reshape(B, Sq, Hq * Dh) @ wo

    def _B_ref(x, k_cache, v_cache, wq, wo):
        B, Sq, D = x.shape
        Hq, Dh = 32, 128
        Hkv, Sk = k_cache.shape[1], k_cache.shape[2]
        W = min(4096, max(256, Sk // 4))
        rep = Hq // Hkv
        q = (lambda x, *d: x.transpose(*d))((x @ wq).reshape(B, Sq, Hq, Dh), 0, 2, 1, 3)
        k = jnp.repeat(k_cache[:, :, Sk - W:, :], rep, axis=1)
        v = jnp.repeat(v_cache[:, :, Sk - W:, :], rep, axis=1)
        scores = jnp.einsum("bhqd,bhkd->bhqk", q, k) * (Dh ** -0.5)
        p = _softmax(scores, axis=-1)
        o = jnp.einsum("bhqk,bhkd->bhqd", p, v)
        return (lambda x, *d: x.transpose(*d))(o, 0, 2, 1, 3).reshape(B, Sq, Hq * Dh) @ wo

    a = _A_ref(A_x, A_k_cache, A_v_cache, A_wq, A_wo)
    b = _B_ref(B_x, B_k_cache, B_v_cache, B_wq, B_wo)
    return jnp.concatenate([a, b], axis=-1)
```

```python
import functools

import jax
import jax.numpy as jnp
from jax import lax
import jax.experimental.pallas as pl
import jax.experimental.pallas.tpu as pltpu

BF16 = jnp.bfloat16
F32 = jnp.float32
NT = (((1,), (1,)), ((), ()))
NN = (((1,), (0,)), ((), ()))


def make(L=8, T=128, interleave=0, checks=False, do_compute=True, flags=None):
    D, HQ, HKV, SK, DH = 576, 32, 16, 8192, 128
    W = min(4096, max(256, SK // 4))
    RA, RB = SK // T, W // T
    NSEM = L + 9
    scale = DH ** -0.5

    def kernel(ax, ak, av, awq, awo, bx, bk, bv, bwq, bwo, out_ref,
               xbuf, wqbuf, wobuf, kbuf, vbuf, q_ref, s_ref, m_ref, l_ref, acc_ref, o_ref, y_ref,
               sems, xsem):
        row = lax.broadcasted_iota(jnp.int32, (8, DH), 0)

        def w_copies(srcs, dst, i, sem):
            c, j = lax.div(i, 8), lax.rem(i, 8)
            col = pl.ds(pl.multiple_of(c * 2048, 2048), 2048)
            cps = []
            for g in range(9):
                r = pl.multiple_of(g * 64 + j * 8, 8)
                for b, src in enumerate(srcs):
                    cps.append(pltpu.make_async_copy(src.at[pl.ds(r, 8), col], dst.at[pl.ds(b * D + r, 8), col], sem))
            return cps

        def kv_copies(src, s0, dst, d0, i, sem):
            cps = []
            for c in range(0, T, 64):
                rs = pl.ds(pl.multiple_of(s0 + i * T + c, 64), 64)
                rd = pl.ds(pl.multiple_of(d0 + i * T + c, 64), 64)
                for h in range(0, HKV, 2):
                    cps.append(pltpu.make_async_copy(src.at[pl.ds(h, 2), rs], dst.at[pl.ds(h, 2), rd], sem))
            return cps

        def w_wait(buf, sem):
            part = buf.at[pl.ds(0, 144), pl.ds(0, 2048)]
            pltpu.make_async_copy(part, part, sem).wait()

        def kv_wait(buf, sem):
            part = buf.at[:, pl.ds(0, T)]
            pltpu.make_async_copy(part, part, sem).wait()

        def q_items(i):
            col = pl.ds(pl.multiple_of(i * 256, 256), 256)
            g, j = lax.div(i, 4), lax.rem(i, 4)
            def item(b):
                x8 = jnp.broadcast_to(xbuf[b, 0].astype(F32), (8, D)).astype(BF16)
                r = lax.dot_general(x8, wqbuf[pl.ds(b * D, D), col], NN, preferred_element_type=F32)
                q = jnp.where(row == 2 * j, r[:, :DH], q_ref[b, g])
                q_ref[b, g] = jnp.where(row == 2 * j + 1, r[:, DH:], q)
            return [functools.partial(item, b) for b in range(2)]

        def k_items(b, d0, i):
            r = d0 // T + i
            rows = pl.ds(pl.multiple_of(r * T, T), T)
            rowt = lax.broadcasted_iota(jnp.int32, (8, T), 0)
            def item(g):
                q8 = q_ref[b, g].astype(BF16)
                s = None
                for j in range(4):
                    sj = lax.dot_general(q8, kbuf[4 * g + j, rows, :], NT, preferred_element_type=F32)
                    s = sj if j == 0 else jnp.where(rowt >= 2 * j, sj, s)
                s = s * scale
                s_ref[r, g] = s
                m = m_ref[b, g]
                for c in range(0, T, DH):
                    m = jnp.maximum(m, s[:, c:c + DH])
                m_ref[b, g] = m
            return [functools.partial(item, g) for g in range(4)]

        def v_items(b, d0, i):
            r = d0 // T + i
            rows = pl.ds(pl.multiple_of(r * T, T), T)
            def item(g):
                m = m_ref[b, g]
                p = jnp.exp(s_ref[r, g] - jnp.concatenate([m] * (T // DH), axis=1))
                l = l_ref[b, g]
                for c in range(0, T, DH):
                    l = l + p[:, c:c + DH]
                l_ref[b, g] = l
                pb = p.astype(BF16)
                o = None
                for j in range(4):
                    oj = lax.dot_general(pb, vbuf[4 * g + j, rows, :], NN, preferred_element_type=F32)
                    o = oj if j == 0 else jnp.where(row >= 2 * j, oj, o)
                acc_ref[b, g] += o
            return [functools.partial(item, g) for g in range(4)]

        def y_items(i):
            col = pl.ds(pl.multiple_of(i * 256, 256), 256)
            def item():
                y_ref[...] += lax.dot_general(o_ref[:, col].astype(BF16), wobuf[:, col], NT, preferred_element_type=F32)
            return [item]

        def finish_max():
            for b in range(2):
                for g in range(4):
                    m_ref[b, g] = jnp.broadcast_to(jnp.max(m_ref[b, g], axis=1, keepdims=True), (8, DH))

        def finish_o():
            for g in range(4):
                o = [acc_ref[b, g] / jnp.sum(l_ref[b, g], axis=1, keepdims=True) for b in range(2)]
                for j in range(8):
                    oa = jnp.broadcast_to(o[0][j:j + 1], (8, DH))
                    ob = jnp.broadcast_to(o[1][j:j + 1], (8, DH))
                    h = 8 * g + j
                    o_ref[:, h * DH:(h + 1) * DH] = jnp.where(row == 0, oa, ob)

        P = functools.partial
        phases = [
            dict(n=16, cp=P(w_copies, (awq, bwq), wqbuf), wait=P(w_wait, wqbuf), items=q_items, grp=8),
            dict(n=RA, cp=P(kv_copies, ak, 0, kbuf, 0), wait=P(kv_wait, kbuf), items=P(k_items, 0, 0), grp=1),
            dict(n=RB, cp=P(kv_copies, bk, SK - W, kbuf, SK), wait=P(kv_wait, kbuf), items=P(k_items, 1, SK), grp=1,
                 post=finish_max),
            dict(n=RA, cp=P(kv_copies, av, 0, vbuf, 0), wait=P(kv_wait, vbuf), items=P(v_items, 0, 0), grp=1),
            dict(n=RB, cp=P(kv_copies, bv, SK - W, vbuf, SK), wait=P(kv_wait, vbuf), items=P(v_items, 1, SK), grp=1,
                 post=finish_o),
            dict(n=16, cp=P(w_copies, (awo, bwo), wobuf), wait=P(w_wait, wobuf), items=y_items, grp=8),
        ]
        starts = [0]
        for p in phases:
            starts.append(starts[-1] + p["n"])
        total = starts[-1]

        def phase_of(t):
            for k in range(len(phases)):
                if t < starts[k + 1]:
                    return k
            return None

        def sem(t):
            return sems.at[lax.rem(t, NSEM)]

        xcps = [pltpu.make_async_copy(src, xbuf.at[pl.ds(b, 1)], xsem.at[b]) for b, src in enumerate((ax, bx))]
        for c in xcps:
            c.start()

        assert L <= 16

        @pl.loop(0, L)
        def _(t):
            for n, c in enumerate(phases[0]["cp"](t, sem(t))):
                c.start(priority=n % 2)

        q_ref[...] = jnp.zeros(q_ref.shape, F32)
        m_ref[...] = jnp.full(m_ref.shape, -jnp.inf, F32)
        l_ref[...] = jnp.zeros(l_ref.shape, F32)
        acc_ref[...] = jnp.zeros(acc_ref.shape, F32)
        y_ref[...] = jnp.zeros(y_ref.shape, F32)
        for c in xcps:
            c.wait()

        cuts = set(starts) | {s - L for s in starts if s - L > 0}
        for k, p in enumerate(phases):
            if p["grp"] > 1:
                cuts |= set(range(starts[k], starts[k + 1], p["grp"]))
        cuts = sorted(cuts)
        for lo, hi in zip(cuts[:-1], cuts[1:]):
            kc, ki = phase_of(lo), phase_of(lo + L)
            pc = phases[kc]
            if pc["grp"] > 1 and (lo - starts[kc]) % pc["grp"] == 0:
                for t in range(lo, lo + pc["grp"]):
                    pc["wait"](sems.at[t % NSEM])

            @pl.loop(lo, hi)
            def _(t):
                cps = phases[ki]["cp"](t + L - starts[ki], sem(t + L)) if ki is not None else []
                if pc["grp"] == 1:
                    pc["wait"](sem(t))
                items = pc["items"](t - starts[kc]) if do_compute else []
                nit = len(items) if interleave and items else 1
                per = -(-len(cps) // nit)
                for n in range(nit):
                    for u in range(n * per, min(len(cps), (n + 1) * per)):
                        cps[u].start(priority=u % 2)
                    for it in (items[n:n + 1] if nit > 1 else items):
                        it()

            if hi == starts[kc + 1] and "post" in pc:
                pc["post"]()

        y = y_ref[...]
        lane = lax.broadcasted_iota(jnp.int32, (1, 2 * D), 1)
        out_ref[0] = jnp.where(lane < D, y[0:1], y[1:2]).astype(out_ref.dtype)

    def f(A_x, A_k, A_v, A_wq, A_wo, B_x, B_k, B_v, B_wq, B_wo):
        hbm = pl.BlockSpec(memory_space=pltpu.HBM)
        kv = lambda a: a.reshape(HKV, SK, DH)
        return pl.pallas_call(
            kernel,
            out_shape=jax.ShapeDtypeStruct((1, 1, 2 * D), A_x.dtype),
            in_specs=[hbm] * 10,
            scratch_shapes=[
                pltpu.VMEM((2, 1, D), BF16),
                pltpu.VMEM((2 * D, HQ * DH), BF16),
                pltpu.VMEM((2 * D, HQ * DH), BF16),
                pltpu.VMEM((HKV, SK + W, DH), BF16),
                pltpu.VMEM((HKV, SK + W, DH), BF16),
                pltpu.VMEM((2, 4, 8, DH), F32),
                pltpu.VMEM((RA + RB, 4, 8, T), F32),
                pltpu.VMEM((2, 4, 8, DH), F32),
                pltpu.VMEM((2, 4, 8, DH), F32),
                pltpu.VMEM((2, 4, 8, DH), F32),
                pltpu.VMEM((8, HQ * DH), F32),
                pltpu.VMEM((8, 2 * D), F32),
                pltpu.SemaphoreType.DMA((NSEM,)),
                pltpu.SemaphoreType.DMA((2,)),
            ],
            compiler_params=pltpu.CompilerParams(
                vmem_limit_bytes=120 * 1024 * 1024,
                disable_bounds_checks=not checks, disable_semaphore_checks=not checks, flags=flags),
        )(A_x, kv(A_k), kv(A_v), A_wq, A_wo.T, B_x, kv(B_k), kv(B_v), B_wq, B_wo.T)

    return f


@jax.jit
def pallas_concat_heads__gqa_block_cached__sliding_block_cached__decode_kernel(
    A_x, A_k_cache, A_v_cache, A_wq, A_wo, B_x, B_k_cache, B_v_cache, B_wq, B_wo):
    return make(L=12, interleave=1)(A_x, A_k_cache, A_v_cache, A_wq, A_wo, B_x, B_k_cache, B_v_cache, B_wq, B_wo)
```

```python
import functools

import jax
import jax.numpy as jnp
from jax import lax
import jax.experimental.pallas as pl
import jax.experimental.pallas.tpu as pltpu

_HQ = 32
_DH = 128
_T = 128
_GRP = 8
_BAND = 8
_STREAMS = 6
_RING = 16
_NT = (((1,), (1,)), ((), ()))
_NN = (((1,), (0,)), ((), ()))


def _dot(a, b, dims):
    return lax.dot_general(a, b, dims, preferred_element_type=jnp.float32)


def _aligned(i, n):
    return i if isinstance(i, int) else pl.multiple_of(i, n)


def _start(copies):
    for n, copy in enumerate(copies):
        copy.start(priority=n % 2)


def _wait(region, sem):
    pltpu.make_async_copy(region, region, sem).wait()


def _overlap(copies, work):
    per = 2 * pl.cdiv(len(copies), 2 * len(work))
    for n, item in enumerate(work):
        _start(copies[n * per:(n + 1) * per])
        item()


def _kernel(ax, ak, av, awq, awo, bx, bk, bv, bwq, bwo, out_ref,
            x_buf, wq_buf, wo_buf, k_buf, v_buf,
            q_ref, s_ref, m_ref, l_ref, acc_ref, o_ref, y_ref,
            x_sems, wq_sem, kv_sems, wo_sems):
    hkv, sk_a, _ = ak.shape
    sk_b = bk.shape[1]
    win = k_buf.shape[1] - sk_a
    d = awq.shape[0]
    half = _HQ * _DH // 2
    rep = _HQ // hkv
    kv_per_grp = _GRP // rep
    ngrp = _HQ // _GRP
    wq, wo = (awq, bwq), (awo, bwo)
    dt = k_buf.dtype
    row = lax.broadcasted_iota(jnp.int32, (_GRP, _DH), 0)

    def w_copy(srcs, dst, b, r, c, sem, nr=_BAND, nc=half):
        col = pl.ds(c, nc)
        return pltpu.make_async_copy(
            srcs[b].at[pl.ds(r, nr), col], dst.at[pl.ds(b * d + r, nr), col], sem)

    def w_round(srcs, dst, i, c, sem):
        return [
            w_copy(srcs, dst, b, _aligned(g * (d // _STREAMS) + i * _BAND, _BAND), c, sem)
            for g in range(_STREAMS) for b in range(2)
        ]

    def kv_round(src, src0, dst, dst0, i, sem):
        copies = []
        for r in range(0, _T, _T // 2):
            rs = pl.ds(_aligned(src0 + i * _T + r, _T // 2), _T // 2)
            rd = pl.ds(_aligned(dst0 + i * _T + r, _T // 2), _T // 2)
            for h in range(0, hkv, 4):
                for heads in (pl.ds(h, 1), pl.ds(h + 1, 3)):
                    copies.append(
                        pltpu.make_async_copy(src.at[heads, rs], dst.at[heads, rd], sem))
        return copies

    def kv_sem(t):
        return kv_sems.at[lax.rem(t, _RING)]

    def q_proj(i, b):
        col = pl.ds(_aligned(i * 4 * _DH, 4 * _DH), 4 * _DH)
        x = jnp.broadcast_to(x_buf[b].astype(jnp.float32), (_GRP, d)).astype(dt)
        res = _dot(x, wq_buf[pl.ds(b * d, d), col], _NN)
        g, r0 = lax.div(i, 2), lax.rem(i, 2) * 4
        q = q_ref[b, g]
        for u in range(4):
            q = jnp.where(row == r0 + u, res[:, u * _DH:(u + 1) * _DH], q)
        q_ref[b, g] = q

    def per_kv_head(lhs, buf, r, g, dims):
        keys = pl.ds(_aligned(r * _T, _T), _T)
        res = _dot(lhs, buf[g * kv_per_grp, keys, :], dims)
        for j in range(1, kv_per_grp):
            res_j = _dot(lhs, buf[g * kv_per_grp + j, keys, :], dims)
            res = jnp.where(row >= j * rep, res_j, res)
        return res

    def scores(b, r, g):
        s = per_kv_head(q_ref[b, g].astype(dt), k_buf, r, g, _NT) * (_DH ** -0.5)
        s_ref[r, g] = s
        m_ref[b, g] = jnp.maximum(m_ref[b, g], s)

    def row_max():
        for b in range(2):
            for g in range(ngrp):
                m = jnp.max(m_ref[b, g], axis=1, keepdims=True)
                m_ref[b, g] = jnp.broadcast_to(m, (_GRP, _T))

    def values(b, r, g):
        p = jnp.exp(s_ref[r, g] - m_ref[b, g])
        l_ref[b, g] += p
        acc_ref[b, g] += per_kv_head(p.astype(dt), v_buf, r, g, _NN)

    def normalize():
        for g in range(ngrp):
            oa, ob = (acc_ref[b, g] / jnp.sum(l_ref[b, g], axis=1, keepdims=True)
                      for b in range(2))
            for j in range(_GRP):
                h = g * _GRP + j
                o_ref[:, h * _DH:(h + 1) * _DH] = jnp.where(row == 0, oa[j:j + 1], ob[j:j + 1])

    def o_proj(r, nr, c, nc):
        col = pl.ds(c, nc)
        return _dot(o_ref[:, col].astype(dt), wo_buf[pl.ds(r, nr), col], _NT)

    def store(blk, y):
        if (blk + 1) * 128 <= d:
            val = y[0:1]
        elif blk * 128 >= d:
            val = y[1:2]
        else:
            lane = lax.broadcasted_iota(jnp.int32, (1, 128), 1)
            val = jnp.where(lane < d - blk * 128, y[0:1], y[1:2])
        out_ref[0, :, blk * 128:(blk + 1) * 128] = val.astype(out_ref.dtype)

    def o_proj_low(c, nc):
        y_ref[...] += o_proj(0, 2 * d, c, nc)

    def o_proj_high(blk, n):
        y = y_ref[:, blk * 128:(blk + n) * 128] + o_proj(blk * 128, n * 128, half, half)
        for u in range(n):
            store(blk + u, y[:, u * 128:(u + 1) * 128])

    rounds = d // _STREAMS // _BAND
    ahead = rounds
    q_steps = _HQ // 4
    assert q_steps <= ahead < _RING

    x_copies = [pltpu.make_async_copy(x, x_buf.at[pl.ds(b, 1)], x_sems.at[b])
                for b, x in enumerate((ax, bx))]
    first = [c for i in range(3) for c in w_round(wq, wq_buf, i, 0, wq_sem)]
    for copy in first[:28]:
        copy.start(priority=1)
    _start(first[28:] + x_copies)

    @pl.loop(3, 2 * rounds)
    def _(i):
        c = _aligned(lax.div(i, rounds) * half, half)
        _start(w_round(wq, wq_buf, lax.rem(i, rounds), c, wq_sem))

    @pl.loop(0, ahead - q_steps)
    def _(t):
        _start(kv_round(ak, 0, k_buf, 0, t, kv_sem(t)))

    for ref in (q_ref, l_ref, acc_ref, y_ref):
        ref[...] = jnp.zeros(ref.shape, ref.dtype)
    m_ref[...] = jnp.full(m_ref.shape, -jnp.inf, m_ref.dtype)
    for copy in x_copies:
        copy.wait()
    _wait(wq_buf, wq_sem)

    @pl.loop(0, q_steps)
    def _(i):
        t = i + ahead - q_steps
        _overlap(kv_round(ak, 0, k_buf, 0, t, kv_sem(t)),
                 [functools.partial(q_proj, i, b) for b in range(2)])

    passes = [
        (sk_a // _T, ak, 0, k_buf, 0, 0, scores),
        (win // _T, bk, sk_b - win, k_buf, sk_a, 1, scores),
        (sk_a // _T, av, 0, v_buf, 0, 0, values),
        (win // _T, bv, sk_b - win, v_buf, sk_a, 1, values),
    ]

    def run_pass(n, t0):
        steps, src, src0, buf, buf0, b, compute = passes[n]
        assert steps >= ahead

        def step(i, copies):
            r = buf0 // _T + i
            _wait(buf.at[:, pl.ds(_aligned(r * _T, _T), _T)], kv_sem(t0 + i))
            _overlap(copies, [functools.partial(compute, b, r, g) for g in range(ngrp)])

        @pl.loop(0, steps - ahead)
        def _(i):
            step(i, kv_round(src, src0, buf, buf0, i + ahead, kv_sem(t0 + i + ahead)))

        @pl.loop(0, ahead)
        def _(i):
            if n + 1 < len(passes):
                copies = kv_round(*passes[n + 1][1:5], i, kv_sem(t0 + steps + i))
            else:
                copies = w_round(wo, wo_buf, i, 0, wo_sems.at[0])
            step(steps - ahead + i, copies)

        return t0 + steps

    t0 = run_pass(1, run_pass(0, 0))
    row_max()
    run_pass(3, run_pass(2, t0))

    def block(blk, s, c=half, nr=_BAND, nc=half):
        return [w_copy(wo, wo_buf, r // d, r % d, c, wo_sems.at[s], nr, nc)
                for r in range(blk * 128, (blk + 1) * 128, nr)]

    def region(blk, n, c=half, nc=half):
        return wo_buf.at[pl.ds(blk * 128, n * 128), pl.ds(c, nc)]

    quarter = half // 2
    last = ((half, 4), (half + quarter, 5))
    early = [c for cs in zip(*(block(blk, 1) for blk in range(5))) for c in cs]
    fast = early[0:48:2] + early[48:] + block(5, 2)
    slow = early[1:48:2] + block(6, 2) + block(7, 3)
    for c, s in last:
        slow += block(8, s, c, 2 * _BAND, quarter)
    assert len(fast) == len(slow)
    copies = [c for pair in zip(fast, slow) for c in pair]

    _start(copies[:32])
    normalize()
    _start(copies[32:80])
    _wait(region(0, 9, 0), wo_sems.at[0])
    _overlap(copies[80:128],
             [functools.partial(o_proj_low, c, 512) for c in range(0, half, 512)])
    _wait(region(0, 5), wo_sems.at[1])
    _overlap(copies[128:], [functools.partial(o_proj_high, blk, 1) for blk in range(5)])
    for blk, n, s in ((5, 2, 2), (7, 1, 3)):
        _wait(region(blk, n), wo_sems.at[s])
        o_proj_high(blk, n)
    y = y_ref[:, 8 * 128:]
    for c, s in last:
        _wait(region(8, 1, c, quarter), wo_sems.at[s])
        y = y + o_proj(8 * 128, 128, c, quarter)
    store(8, y)


@jax.jit
def pallas_concat_heads__gqa_block_cached__sliding_block_cached__decode_kernel(
    A_x: jax.Array,
    A_k_cache: jax.Array,
    A_v_cache: jax.Array,
    A_wq: jax.Array,
    A_wo: jax.Array,
    B_x: jax.Array,
    B_k_cache: jax.Array,
    B_v_cache: jax.Array,
    B_wq: jax.Array,
    B_wo: jax.Array,
):
    d = A_x.shape[-1]
    _, hkv, sk_a, _ = A_k_cache.shape
    sk_b = B_k_cache.shape[2]
    win = min(4096, max(256, sk_b // 4))
    assert A_x.shape == B_x.shape == (1, 1, d) and 2 * d == 9 * 128 and hkv % 4 == 0
    assert sk_a % _T == 0 and sk_b % _T == 0 and win % _T == 0 and win <= sk_b
    dt = A_k_cache.dtype
    keys = sk_a + win
    per_head = pltpu.VMEM((2, _HQ // _GRP, _GRP, _DH), jnp.float32)

    def cache(a):
        return a.reshape(a.shape[1:])

    return pl.pallas_call(
        _kernel,
        out_shape=jax.ShapeDtypeStruct((1, 1, 2 * d), A_x.dtype),
        in_specs=[pl.BlockSpec(memory_space=pltpu.HBM)] * 10,
        scratch_shapes=[
            pltpu.VMEM((2, 1, d), dt),
            pltpu.VMEM((2 * d, _HQ * _DH), dt),
            pltpu.VMEM((2 * d, _HQ * _DH), dt),
            pltpu.VMEM((hkv, keys, _DH), dt),
            pltpu.VMEM((hkv, keys, _DH), dt),
            per_head,
            pltpu.VMEM((keys // _T, _HQ // _GRP, _GRP, _T), jnp.float32),
            per_head,
            per_head,
            per_head,
            pltpu.VMEM((_GRP, _HQ * _DH), jnp.float32),
            pltpu.VMEM((_GRP, 2 * d), jnp.float32),
            pltpu.SemaphoreType.DMA((2,)),
            pltpu.SemaphoreType.DMA(()),
            pltpu.SemaphoreType.DMA((_RING,)),
            pltpu.SemaphoreType.DMA((6,)),
        ],
        compiler_params=pltpu.CompilerParams(
            vmem_limit_bytes=112 * 1024 * 1024,
            disable_semaphore_checks=True,
        ),
    )(A_x, cache(A_k_cache), cache(A_v_cache), A_wq, A_wo.T,
      B_x, cache(B_k_cache), cache(B_v_cache), B_wq, B_wo.T)
```
